```python
import os as _os
_os.environ.setdefault("JAX_PLATFORMS", "cpu")
import jax
import jax.numpy as jnp

def _softmax(x, axis=-1):
    return jax.nn.softmax(x, axis=axis)
def _gelu(x):
    return jax.nn.gelu(x, approximate=True)
def _silu(x):
    return jax.nn.silu(x)
def _sigmoid(x):
    return jax.nn.sigmoid(x)
def _layernorm(x, axis=-1, eps=1e-5):
    m = jnp.mean(x, axis=axis, keepdims=True)
    v = jnp.var(x, axis=axis, keepdims=True)
    return (x - m) / jnp.sqrt(v + eps)
def _scatter_add(tgt, idx, src, axis=0):
    return tgt.at[idx].add(src)
def _segment_sum(src, seg, n):
    return jax.ops.segment_sum(src, seg, n)
class _Rng:
    def __init__(self, key):
        self._k = key
    def _next(self):
        self._k, sub = jax.random.split(self._k)
        return sub
    def normal(self, shape):
        return jax.random.normal(self._next(), shape, dtype=jnp.bfloat16)
    def randint(self, lo, hi, shape):
        return jax.random.randint(self._next(), shape, lo, hi, dtype=jnp.int32)
    def uniform(self, shape, lo=0.0, hi=1.0):
        return jax.random.uniform(self._next(), shape, jnp.bfloat16, lo, hi)
    def permutation(self, n):
        return jax.random.permutation(self._next(), n)


kernel_name = 'concat_heads__gqa_block_cached__gqa_block_cached__near_ridge'

def setup_inputs():
    _rng = _Rng(jax.random.key(int.from_bytes(__import__("os").urandom(4), "little")))
    _w = (lambda a: (lambda t: t.astype(jnp.bfloat16) if jnp.issubdtype(t.dtype, jnp.floating) else t)(jnp.asarray(a)))
    def _A_setup():
        B, Sq, D = 8, 240, 640
        Hq, Hkv, Sk, Dh = 32, 32, 1024, 192
        assert Hq % Hkv == 0, (Hq, Hkv)
        return {
            "x": _w((lambda *s: _rng.normal(s) * 0.8)(B, Sq, D)),
            "k_cache": _w((lambda *s: _rng.normal(s) * 0.8)(B, Hkv, Sk, Dh)),
            "v_cache": _w((lambda *s: _rng.normal(s) * 0.05)(B, Hkv, Sk, Dh)),
            "wq": _w((lambda *s: _rng.normal(s) * 0.8)(D, Hq * Dh) * (D ** -0.5)),
            "wo": _w((lambda *s: _rng.normal(s) * 0.05)(Hq * Dh, D) * ((Hq * Dh) ** -0.5)),
        }
    _A_in = _A_setup()

    def _B_setup():
        B, Sq, D = 8, 240, 640
        Hq, Hkv, Sk, Dh = 32, 32, 1024, 192
        assert Hq % Hkv == 0, (Hq, Hkv)
        return {
            "x": _w((lambda *s: _rng.normal(s) * 0.8)(B, Sq, D)),
            "k_cache": _w((lambda *s: _rng.normal(s) * 0.8)(B, Hkv, Sk, Dh)),
            "v_cache": _w((lambda *s: _rng.normal(s) * 0.05)(B, Hkv, Sk, Dh)),
            "wq": _w((lambda *s: _rng.normal(s) * 0.8)(D, Hq * Dh) * (D ** -0.5)),
            "wo": _w((lambda *s: _rng.normal(s) * 0.05)(Hq * Dh, D) * ((Hq * Dh) ** -0.5)),
        }
    _B_in = _B_setup()

    return {
        "A_x": _A_in["x"],
        "A_k_cache": _A_in["k_cache"],
        "A_v_cache": _A_in["v_cache"],
        "A_wq": _A_in["wq"],
        "A_wo": _A_in["wo"],
        "B_x": _B_in["x"],
        "B_k_cache": _B_in["k_cache"],
        "B_v_cache": _B_in["v_cache"],
        "B_wq": _B_in["wq"],
        "B_wo": _B_in["wo"],
    }

def reference(A_x, A_k_cache, A_v_cache, A_wq, A_wo, B_x, B_k_cache, B_v_cache, B_wq, B_wo):
    def _A_ref(x, k_cache, v_cache, wq, wo):
        B, Sq, D = x.shape
        Hq, Dh = 32, 192
        Hkv = k_cache.shape[1]
        rep = Hq // Hkv
        q = (lambda x, *d: x.transpose(*d))((x @ wq).reshape(B, Sq, Hq, Dh), 0, 2, 1, 3)
        k = jnp.repeat(k_cache, rep, axis=1)
        v = jnp.repeat(v_cache, rep, axis=1)
        scores = jnp.einsum("bhqd,bhkd->bhqk", q, k) * (Dh ** -0.5)
        p = _softmax(scores, axis=-1)
        o = jnp.einsum("bhqk,bhkd->bhqd", p, v)
        return (lambda x, *d: x.transpose(*d))(o, 0, 2, 1, 3).reshape(B, Sq, Hq * Dh) @ wo

    def _B_ref(x, k_cache, v_cache, wq, wo):
        B, Sq, D = x.shape
        Hq, Dh = 32, 192
        Hkv = k_cache.shape[1]
        rep = Hq // Hkv
        q = (lambda x, *d: x.transpose(*d))((x @ wq).reshape(B, Sq, Hq, Dh), 0, 2, 1, 3)
        k = jnp.repeat(k_cache, rep, axis=1)
        v = jnp.repeat(v_cache, rep, axis=1)
        scores = jnp.einsum("bhqd,bhkd->bhqk", q, k) * (Dh ** -0.5)
        p = _softmax(scores, axis=-1)
        o = jnp.einsum("bhqk,bhkd->bhqd", p, v)
        return (lambda x, *d: x.transpose(*d))(o, 0, 2, 1, 3).reshape(B, Sq, Hq * Dh) @ wo

    a = _A_ref(A_x, A_k_cache, A_v_cache, A_wq, A_wo)
    b = _B_ref(B_x, B_k_cache, B_v_cache, B_wq, B_wo)
    return jnp.concatenate([a, b], axis=-1)
```

```python
import jax
import jax.numpy as jnp
import jax.experimental.pallas as pl
import jax.experimental.pallas.tpu as pltpu

B, SQ, D = 8, 240, 640
H, SK, DH = 32, 1024, 192
NP = H // 2
LOG2E = 1.4426950408889634
C = (DH ** -0.5) * LOG2E
NT = (((1,), (1,)), ((), ()))
F32, BF16 = jnp.float32, jnp.bfloat16
RC = 16
NRC = SQ // RC
NKT = SK // 128
NB = 2
NG = B // NB
LAST = NP * NG - 1
OSPLIT = 256
QEARLY = True
LMODE = 'B'


def _kernel(xa_h, ka_h, va_h, wqa_h, woa_h, xb_h, kb_h, vb_h, wqb_h, wob_h, o_hbm,
            acc_ref, x_buf, kv_buf, wq_buf, wo_buf, o_buf, kv_sem, x_sem, w_sem, o_sem):
    x_h, wq_h, wo_h = (xa_h, xb_h), (wqa_h, wqb_h), (woa_h, wob_h)
    kv_h = ((ka_h, va_h), (kb_h, vb_h))

    def start_data(it):
        sl, p, b0 = it % 2, it // NG, (it % NG) * NB
        for br in range(2):
            pltpu.make_async_copy(x_h[br].at[pl.ds(b0, NB)], x_buf.at[sl, br], x_sem.at[sl]).start()
            for kv in range(2):
                pltpu.make_async_copy(kv_h[br][kv].at[pl.ds(b0, NB), pl.ds(2 * p, 2)],
                                      kv_buf.at[sl, br, kv], kv_sem.at[sl]).start()

    def wait_data(it):
        sl = it % 2
        pltpu.make_async_copy(x_buf.at[sl], x_buf.at[sl], x_sem.at[sl]).wait()
        pltpu.make_async_copy(kv_buf.at[sl], kv_buf.at[sl], kv_sem.at[sl]).wait()

    def start_w(p):
        sl = p % 2
        cols = pl.ds(pl.multiple_of(p * (2 * DH), 2 * DH), 2 * DH)
        for br in range(2):
            pltpu.make_async_copy(wq_h[br].at[:, cols], wq_buf.at[sl, br], w_sem.at[sl, 0]).start()
            pltpu.make_async_copy(wo_h[br].at[cols, :], wo_buf.at[sl, br], w_sem.at[sl, 1]).start()

    def wait_w(p):
        sl = p % 2
        pltpu.make_async_copy(wq_buf.at[sl], wq_buf.at[sl], w_sem.at[sl, 0]).wait()
        pltpu.make_async_copy(wo_buf.at[sl], wo_buf.at[sl], w_sem.at[sl, 1]).wait()

    def o_copy(bi):
        return pltpu.make_async_copy(o_buf.at[bi], o_hbm.at[bi], o_sem.at[bi])

    class Head:
        def __init__(self, k_ref, v_ref, h):
            self.q, self.k_ref, self.v_ref, self.h = None, k_ref, v_ref, h
            self.s = [None] * 4
            self.p = [None] * NRC
            self.r = [None] * NRC
            self.o = [None, None]

        def s_round(self, j):
            cols = slice(256 * j, 256 * (j + 1))
            z = jnp.zeros((64, 256), BF16)
            if self.h == 0:
                lhs, rhs = self.q[:, 0:256], jnp.concatenate([self.k_ref[0, :, cols], z], 0)
            else:
                lhs, rhs = self.q[:, 128:384], jnp.concatenate([z, self.k_ref[1, :, cols]], 0)
            self.s[j] = jnp.dot(lhs, rhs, preferred_element_type=F32)

        def sm_chunk(self, r):
            rows = slice(RC * r, RC * (r + 1))
            s = [self.s[j // 2][rows, 128 * (j % 2):128 * (j % 2 + 1)] for j in range(NKT)]
            mx = s[0]
            for t in s[1:]:
                mx = jnp.maximum(mx, t)
            m = jnp.max(mx, axis=1, keepdims=True)
            e = [jnp.exp2(t - m) for t in s]
            self.p[r] = [t.astype(BF16) for t in e]
            src = [t.astype(F32) for t in self.p[r]] if LMODE == 'O' else e
            l = src[0]
            for t in src[1:]:
                l = l + t
            self.r[r] = jnp.broadcast_to(1.0 / jnp.sum(l, axis=1, keepdims=True), (RC, 128))

        def pv_round(self, j):
            n, kh = divmod(j, 2)
            chunks = range(0, 8) if n == 0 else range(8, NRC)
            rhs = jnp.concatenate(
                [jnp.concatenate(self.p[r][4 * kh:4 * kh + 4], axis=1) for r in chunks], axis=0)
            o = jax.lax.dot_general(self.v_ref[self.h, :, 512 * kh:512 * (kh + 1)], rhs, NT,
                                    preferred_element_type=F32)
            self.o[n] = o if kh == 0 else self.o[n] + o

        S = property(lambda self: [(lambda j=j: self.s_round(j)) for j in range(4)])
        SM = property(lambda self: [(lambda r=r: self.sm_chunk(r)) for r in range(NRC)])
        PV = property(lambda self: [(lambda j=j: self.pv_round(j)) for j in range(4)])

    def interleave(rounds, chunks=()):
        per = -(-len(chunks) // len(rounds)) if chunks else 0
        for i, f in enumerate(rounds):
            f()
            for c in chunks[i * per:(i + 1) * per]:
                c()

    def compute(p, g):
        it = p * NG + g
        slot, ws = it % 2, p % 2
        units = [(bb, br) for bb in range(NB) for br in range(2)]
        heads = [Head(kv_buf.at[slot, br, 0, bb], kv_buf.at[slot, br, 1, bb], h)
                 for bb, br in units for h in range(2)]
        U = len(units)
        NH = 2 * U
        o_pair = [None] * U

        def qproj(u):
            bb, br = units[u]
            q = jnp.dot(x_buf[slot, br, bb], wq_buf[ws, br], preferred_element_type=F32)
            heads[2 * u].q = heads[2 * u + 1].q = (q * C).astype(BF16)

        def outproj(u, cols=slice(0, D)):
            bb, br = units[u]
            if o_pair[u] is None:
                h0, h1 = heads[2 * u], heads[2 * u + 1]
                o = jnp.concatenate([jnp.concatenate([h0.o[n], h1.o[n]], axis=0).T for n in range(2)], axis=0)
                r0, r1 = jnp.concatenate(h0.r, axis=0), jnp.concatenate(h1.r, axis=0)
                lo = jax.lax.broadcasted_iota(jnp.int32, (SQ, 128), 1) < 64
                o_pair[u] = jnp.concatenate([o[:, 0:128] * r0, o[:, 128:256] * jnp.where(lo, r0, r1),
                                             o[:, 256:384] * r1], axis=1).astype(BF16)
            y = jnp.dot(o_pair[u], wo_buf[ws, br, :, cols], preferred_element_type=F32)
            bi = g * NB + bb
            acc_ref[br, bi, :, cols] = jnp.where(p == 0, 0.0, acc_ref[br, bi, :, cols]) + y

        qproj(0)
        qproj(1)
        interleave(heads[0].S)
        for t in range(NH):
            if t + 1 < NH:
                interleave(heads[t + 1].S, heads[0].SM if t == 0 else ())
                if QEARLY and t % 2 == 0 and t // 2 + 2 < U:
                    qproj(t // 2 + 2)
                if not QEARLY and (t + 1) % 2 == 0 and (t + 1) // 2 + 1 < U:
                    qproj((t + 1) // 2 + 1)
            if t == NH - 1 and OSPLIT > 0:
                outproj(U - 2, slice(0, OSPLIT))
            interleave(heads[t].PV, heads[t + 1].SM if t + 1 < NH else ())
            if t % 2 == 0 and t >= 2 and t // 2 - 1 <= U - 3:
                outproj(t // 2 - 1)
        if OSPLIT < D:
            outproj(U - 2, slice(OSPLIT, D))
        outproj(U - 1)

        @pl.when(it + 2 <= LAST)
        def _prefetch():
            start_data(it + 2)

        @pl.when(p == NP - 1)
        def _emit():
            for bb in range(NB):
                bi = g * NB + bb
                for br in range(2):
                    o_buf[bi, :, br * D:(br + 1) * D] = acc_ref[br, bi].astype(BF16)
                o_copy(bi).start()

        @pl.when(it + 1 <= LAST)
        def _next():
            wait_data(it + 1)

    start_w(0)
    start_data(0)
    wait_w(0)
    wait_data(0)
    start_data(1)
    start_w(1)

    def pair_step(p, carry):
        jax.lax.fori_loop(0, NG, lambda g, c: (compute(p, g), c)[1], 0)

        @pl.when(p + 2 < NP)
        def _():
            start_w(p + 2)

        @pl.when(p + 1 < NP)
        def _():
            wait_w(p + 1)
        return carry

    jax.lax.fori_loop(0, NP, pair_step, 0)
    for bi in range(B):
        o_copy(bi).wait()


@jax.jit
def pallas_concat_heads__gqa_block_cached__gqa_block_cached__near_ridge_kernel(
    A_x, A_k_cache, A_v_cache, A_wq, A_wo, B_x, B_k_cache, B_v_cache, B_wq, B_wo):
    t = lambda a: jnp.swapaxes(a, 2, 3)
    hbm = pl.BlockSpec(memory_space=pl.ANY)
    dma = pltpu.SemaphoreType.DMA
    return pl.pallas_call(
        _kernel,
        in_specs=[hbm] * 10,
        out_specs=hbm,
        out_shape=jax.ShapeDtypeStruct((B, SQ, 2 * D), BF16),
        scratch_shapes=[
            pltpu.VMEM((2, B, SQ, D), F32),
            pltpu.VMEM((2, 2, NB, SQ, D), BF16),
            pltpu.VMEM((2, 2, 2, NB, 2, DH, SK), BF16),
            pltpu.VMEM((2, 2, D, 2 * DH), BF16),
            pltpu.VMEM((2, 2, 2 * DH, D), BF16),
            pltpu.VMEM((B, SQ, 2 * D), BF16),
            dma((2,)), dma((2,)), dma((2, 2)), dma((B,)),
        ],
        compiler_params=pltpu.CompilerParams(
            vmem_limit_bytes=100 * 1024 * 1024, disable_bounds_checks=True),
    )(A_x, t(A_k_cache), t(A_v_cache), A_wq, A_wo, B_x, t(B_k_cache), t(B_v_cache), B_wq, B_wo)
```

```python
import jax
import jax.numpy as jnp
import jax.experimental.pallas as pl
import jax.experimental.pallas.tpu as pltpu

B, SQ, D = 8, 240, 640
H, SK, DH = 32, 1024, 192
NP = H // 2
PW = 2 * DH
NB = 4
NG = B // NB
NIT = (NP - 1) * NG
RC = 16
NRC = SQ // RC
NKT = SK // 128
OSPLIT = 256
SCALE = (DH ** -0.5) * 1.4426950408889634
NT = (((1,), (1,)), ((), ()))
F32, BF16 = jnp.float32, jnp.bfloat16


class _Head:
    def __init__(self, k_ref, v_ref, h):
        self.k_ref, self.v_ref, self.h = k_ref, v_ref, h
        self.q = None
        self.s = None
        self.p = [None] * NRC
        self.r = [None] * NRC
        self.o = None

    def scores(self):
        z = jnp.zeros((64, SK), BF16)
        if self.h == 0:
            lhs, rhs = self.q[:, 0:256], jnp.concatenate([self.k_ref[0], z], 0)
        else:
            lhs, rhs = self.q[:, 128:384], jnp.concatenate([z, self.k_ref[1]], 0)
        self.s = jnp.dot(lhs, rhs, preferred_element_type=F32)

    def softmax(self):
        for c in range(NRC):
            rows = slice(RC * c, RC * (c + 1))
            s = [self.s[rows, 128 * j:128 * (j + 1)] for j in range(NKT)]
            mx = s[0]
            for t in s[1:]:
                mx = jnp.maximum(mx, t)
            m = jnp.max(mx, axis=1, keepdims=True)
            e = [jnp.exp2(t - m) for t in s]
            self.p[c] = [t.astype(BF16) for t in e]
            l = e[0]
            for t in e[1:]:
                l = l + t
            self.r[c] = jnp.broadcast_to(1.0 / jnp.sum(l, axis=1, keepdims=True), (RC, 128))

    def pv(self):
        p = jnp.concatenate([jnp.concatenate(tiles, axis=1) for tiles in self.p], axis=0)
        self.o = jax.lax.dot_general(self.v_ref[self.h], p, NT, preferred_element_type=F32)


def _kernel(xa_h, ka_h, va_h, wqa_h, woa_h, xb_h, kb_h, vb_h, wqb_h, wob_h, o_hbm,
            acc_ref, x_buf, kvw_buf, kv_buf, wq_buf, wo_buf, o_buf,
            warm_sem, kv_sem, w_sem, o_sem, first_sem):
    x_h, wq_h, wo_h = (xa_h, xb_h), (wqa_h, wqb_h), (woa_h, wob_h)
    kv_h = ((ka_h, va_h), (kb_h, vb_h))

    def wait_all(buf, sem):
        pltpu.make_async_copy(buf, buf, sem).wait()

    def start_warm(b):
        sl = b % 2
        for br in range(2):
            pltpu.make_async_copy(x_h[br].at[b], x_buf.at[b, br], warm_sem.at[sl, 0]).start()
            for kv in range(2):
                pltpu.make_async_copy(kv_h[br][kv].at[b, pl.ds(0, 2)], kvw_buf.at[sl, br, kv],
                                      warm_sem.at[sl, 1]).start()

    def wait_warm(b):
        sl = b % 2
        wait_all(x_buf.at[b], warm_sem.at[sl, 0])
        wait_all(kvw_buf.at[sl], warm_sem.at[sl, 1])

    def start_main(it):
        sl, p, b0 = it % 2, 1 + it // NG, (it % NG) * NB
        for br in range(2):
            for kv in range(2):
                pltpu.make_async_copy(kv_h[br][kv].at[pl.ds(b0, NB), pl.ds(2 * p, 2)],
                                      kv_buf.at[sl, br, kv], kv_sem.at[sl]).start()

    def start_main_piece(j):
        bb, h = j // 2, j % 2
        for br in range(2):
            for kv in range(2):
                pltpu.make_async_copy(kv_h[br][kv].at[bb, 2 + h], kv_buf.at[0, br, kv, bb, h],
                                      kv_sem.at[0]).start()

    def wait_main(it):
        sl = it % 2
        wait_all(kv_buf.at[sl], kv_sem.at[sl])

    def start_w(p, which=(0, 1)):
        sl = p % 2
        cols = pl.ds(pl.multiple_of(p * PW, PW), PW)
        for br in range(2):
            if 0 in which:
                pltpu.make_async_copy(wq_h[br].at[:, cols], wq_buf.at[sl, br], w_sem.at[sl, 0]).start()
            if 1 in which:
                pltpu.make_async_copy(wo_h[br].at[cols, :], wo_buf.at[sl, br], w_sem.at[sl, 1]).start()

    def wait_w(p, which=(0, 1)):
        sl = p % 2
        if 0 in which:
            wait_all(wq_buf.at[sl], w_sem.at[sl, 0])
        if 1 in which:
            wait_all(wo_buf.at[sl], w_sem.at[sl, 1])

    def o_copy(bi):
        return pltpu.make_async_copy(o_buf.at[bi], o_hbm.at[bi], o_sem.at[bi])

    def compute(nb, b0, kv_view, ws, first, final=None, mid=None):
        units = [(bb, br) for bb in range(nb) for br in range(2)]
        heads = [_Head(kv_view(br, 0, bb), kv_view(br, 1, bb), h) for bb, br in units for h in range(2)]
        nu = len(units)
        nh = 2 * nu
        o_pair = [None] * nu

        def qproj(u):
            bb, br = units[u]
            q = jnp.dot(x_buf[b0 + bb, br], wq_buf[ws, br], preferred_element_type=F32)
            heads[2 * u].q = heads[2 * u + 1].q = (q * SCALE).astype(BF16)

        def outproj(u, cols=slice(0, D)):
            bb, br = units[u]
            if o_pair[u] is None:
                h0, h1 = heads[2 * u], heads[2 * u + 1]
                o = jnp.concatenate([h0.o, h1.o], axis=0).T
                r0, r1 = jnp.concatenate(h0.r, axis=0), jnp.concatenate(h1.r, axis=0)
                lo = jax.lax.broadcasted_iota(jnp.int32, (SQ, 128), 1) < 64
                o_pair[u] = jnp.concatenate([o[:, 0:128] * r0, o[:, 128:256] * jnp.where(lo, r0, r1),
                                             o[:, 256:384] * r1], axis=1).astype(BF16)
            y = jnp.dot(o_pair[u], wo_buf[ws, br, :, cols], preferred_element_type=F32)
            if first:
                acc_ref[br, b0 + bb, :, cols] = y
            else:
                y = acc_ref[br, b0 + bb, :, cols] + y
                acc_ref[br, b0 + bb, :, cols] = y
                o_buf[b0 + bb, :, br * D + cols.start:br * D + cols.stop] = y.astype(BF16)
                if br == 1 and cols.stop == D:
                    @pl.when(final)
                    def _():
                        o_copy(b0 + bb).start()

        qproj(0)
        qproj(1)
        heads[0].scores()
        for t in range(nh):
            if t == 1 and mid is not None:
                mid()
            if t + 1 < nh:
                heads[t + 1].scores()
                if t % 2 == 0 and t // 2 + 2 < nu:
                    qproj(t // 2 + 2)
            heads[t].softmax()
            if t == nh - 1:
                outproj(nu - 2, slice(0, OSPLIT))
            heads[t].pv()
            if t % 2 == 0 and t >= 2 and t // 2 - 1 <= nu - 3:
                outproj(t // 2 - 1)
        outproj(nu - 2, slice(OSPLIT, D))
        outproj(nu - 1)

    def start_first_kv(br):
        for kv in range(2):
            pltpu.make_async_copy(kv_h[br][kv].at[0, pl.ds(0, 2)], kvw_buf.at[0, br, kv],
                                  first_sem.at[br]).start()

    for br in range(2):
        pltpu.make_async_copy(x_h[br].at[0], x_buf.at[0, br], warm_sem.at[0, 0]).start()
    start_w(0, which=(0,))
    start_first_kv(0)
    wait_all(x_buf.at[0], warm_sem.at[0, 0])
    wait_w(0, which=(0,))
    wait_all(kvw_buf.at[0, 0], first_sem.at[0])
    start_first_kv(1)
    start_w(0, which=(1,))

    def mid():
        wait_all(kvw_buf.at[0, 1], first_sem.at[1])
        wait_w(0, which=(1,))
        start_warm(1)

    compute(1, 0, lambda br, kv, bb: kvw_buf.at[0, br, kv], 0, True, mid=mid)
    start_warm(2)
    start_main_piece(0)
    wait_warm(1)

    def warm_step(b, carry):
        sl = b % 2
        compute(1, b, lambda br, kv, bb: kvw_buf.at[sl, br, kv], 0, True)

        @pl.when(b + 2 < B)
        def _():
            start_warm(b + 2)

        @pl.when(b < B - 1)
        def _():
            start_main_piece(b)

        @pl.when(b == B - 2)
        def _():
            start_main_piece(B - 1)
            start_w(1)

        @pl.when(b + 1 < B)
        def _():
            wait_warm(b + 1)
        return carry

    jax.lax.fori_loop(1, B, warm_step, 0)
    wait_w(1)
    wait_main(0)
    start_main(1)
    start_w(2)

    def main_step(p, g):
        it = (p - 1) * NG + g
        sl = it % 2
        compute(NB, g * NB, lambda br, kv, bb: kv_buf.at[sl, br, kv, bb], p % 2, False,
                final=p == NP - 1)

        @pl.when(it + 2 < NIT)
        def _():
            start_main(it + 2)

        @pl.when(it + 1 < NIT)
        def _():
            wait_main(it + 1)

    def pair_step(p, carry):
        jax.lax.fori_loop(0, NG, lambda g, c: (main_step(p, g), c)[1], 0)

        @pl.when(p + 2 < NP)
        def _():
            start_w(p + 2)

        @pl.when(p + 1 < NP)
        def _():
            wait_w(p + 1)
        return carry

    jax.lax.fori_loop(1, NP, pair_step, 0)
    for bi in range(B):
        o_copy(bi).wait()


@jax.jit
def pallas_concat_heads__gqa_block_cached__gqa_block_cached__near_ridge_kernel(
    A_x: jax.Array,
    A_k_cache: jax.Array,
    A_v_cache: jax.Array,
    A_wq: jax.Array,
    A_wo: jax.Array,
    B_x: jax.Array,
    B_k_cache: jax.Array,
    B_v_cache: jax.Array,
    B_wq: jax.Array,
    B_wo: jax.Array,
):
    assert A_x.shape == B_x.shape == (B, SQ, D)
    assert A_k_cache.shape == A_v_cache.shape == B_k_cache.shape == B_v_cache.shape == (B, H, SK, DH)
    assert A_wq.shape == B_wq.shape == (D, H * DH) and A_wo.shape == B_wo.shape == (H * DH, D)

    t = lambda a: jnp.swapaxes(a, 2, 3)
    hbm = pl.BlockSpec(memory_space=pl.ANY)
    dma = pltpu.SemaphoreType.DMA
    return pl.pallas_call(
        _kernel,
        in_specs=[hbm] * 10,
        out_specs=hbm,
        out_shape=jax.ShapeDtypeStruct((B, SQ, 2 * D), A_x.dtype),
        scratch_shapes=[
            pltpu.VMEM((2, B, SQ, D), F32),
            pltpu.VMEM((B, 2, SQ, D), BF16),
            pltpu.VMEM((2, 2, 2, 2, DH, SK), BF16),
            pltpu.VMEM((2, 2, 2, NB, 2, DH, SK), BF16),
            pltpu.VMEM((2, 2, D, PW), BF16),
            pltpu.VMEM((2, 2, PW, D), BF16),
            pltpu.VMEM((B, SQ, 2 * D), BF16),
            dma((2, 2)), dma((2,)), dma((2, 2)), dma((B,)), dma((2,)),
        ],
        compiler_params=pltpu.CompilerParams(
            vmem_limit_bytes=100 * 1024 * 1024,
            disable_bounds_checks=True,
        ),
    )(A_x, t(A_k_cache), t(A_v_cache), A_wq, A_wo, B_x, t(B_k_cache), t(B_v_cache), B_wq, B_wo)
```
